```python
import os as _os
_os.environ.setdefault("JAX_PLATFORMS", "cpu")
import jax
import jax.numpy as jnp

def _softmax(x, axis=-1):
    return jax.nn.softmax(x, axis=axis)
def _gelu(x):
    return jax.nn.gelu(x, approximate=True)
def _silu(x):
    return jax.nn.silu(x)
def _sigmoid(x):
    return jax.nn.sigmoid(x)
def _layernorm(x, axis=-1, eps=1e-5):
    m = jnp.mean(x, axis=axis, keepdims=True)
    v = jnp.var(x, axis=axis, keepdims=True)
    return (x - m) / jnp.sqrt(v + eps)
def _scatter_add(tgt, idx, src, axis=0):
    return tgt.at[idx].add(src)
def _segment_sum(src, seg, n):
    return jax.ops.segment_sum(src, seg, n)
class _Rng:
    def __init__(self, key):
        self._k = key
    def _next(self):
        self._k, sub = jax.random.split(self._k)
        return sub
    def normal(self, shape):
        return jax.random.normal(self._next(), shape, dtype=jnp.bfloat16)
    def randint(self, lo, hi, shape):
        return jax.random.randint(self._next(), shape, lo, hi, dtype=jnp.int32)
    def uniform(self, shape, lo=0.0, hi=1.0):
        return jax.random.uniform(self._next(), shape, jnp.bfloat16, lo, hi)
    def permutation(self, n):
        return jax.random.permutation(self._next(), n)


kernel_name = 'standalone__mha_softmax__near_ridge'

def setup_inputs():
    _rng = _Rng(jax.random.key(int.from_bytes(__import__("os").urandom(4), "little")))
    _w = (lambda a: (lambda t: t.astype(jnp.bfloat16) if jnp.issubdtype(t.dtype, jnp.floating) else t)(jnp.asarray(a)))
    B, H, Sq, Sk, D = 16, 16, 256, 256, 256
    return {
        "q": _w((lambda *s: _rng.normal(s) * 0.4)(B, H, Sq, D)),
        "k": _w((lambda *s: _rng.normal(s) * 0.4)(B, H, Sk, D)),
        "v": _w((lambda *s: _rng.normal(s) * 0.05)(B, H, Sk, D)),
    }

def reference(q, k, v):
    scale = q.shape[-1] ** -0.5
    scores = jnp.einsum("bhqd,bhkd->bhqk", q, k) * scale
    p = _softmax(scores, axis=-1)
    return jnp.einsum("bhqk,bhkd->bhqd", p, v)
```

```python
import jax
import jax.numpy as jnp
import jax.experimental.pallas as pl
import jax.experimental.pallas.tpu as pltpu

_HEADS_PER_CHUNK = 2
_RING_DEPTH = 4
_WRITE_LEAD = 2
_NT = (((1,), (1,)), ((), ()))


def _attention_head(q, k, v, scale):
    s = jax.lax.dot_general(q, k, _NT, preferred_element_type=jnp.float32)
    m = jnp.max(s, axis=-1, keepdims=True)
    p = jnp.exp((s - m) * scale)
    l = jnp.sum(p, axis=-1, keepdims=True)
    o = jnp.dot(p.astype(v.dtype), v, preferred_element_type=jnp.float32)
    return o * (1.0 / l)


def _kernel(q_hbm, k_hbm, v_hbm, o_hbm, q_buf, k_buf, v_buf, o_buf, r_sem, w_sem, *, hb, depth, lead):
    n = q_hbm.shape[0] // hb
    scale = q_hbm.shape[-1] ** -0.5

    def reads(i, slot):
        return [
            pltpu.make_async_copy(src.at[pl.ds(i * hb, hb)], dst.at[slot], r_sem.at[j, slot])
            for j, (src, dst) in enumerate(((q_hbm, q_buf), (k_hbm, k_buf), (v_hbm, v_buf)))
        ]

    def write(start, size):
        return pltpu.make_async_copy(
            o_buf.at[pl.ds(start, size)], o_hbm.at[pl.ds(start, size)], w_sem.at[0])

    for i in range(min(depth - 1, n)):
        for c in reads(i, i):
            c.start()

    w0 = max(n - lead, 0)

    def body(i, carry):
        slot = jax.lax.rem(i, depth)
        nxt = i + depth - 1

        @pl.when(nxt < n)
        def _():
            for c in reads(nxt, jax.lax.rem(nxt, depth)):
                c.start()

        for c in reads(i, slot):
            c.wait()

        if w0 > 0:
            @pl.when(i == w0)
            def _():
                write(0, w0 * hb).start()

        @pl.when(i > w0)
        def _():
            write((i - 1) * hb, hb).start()

        for h in range(hb):
            o = _attention_head(q_buf[slot, h], k_buf[slot, h], v_buf[slot, h], scale)
            o_buf[i * hb + h] = o.astype(o_buf.dtype)
        return carry

    jax.lax.fori_loop(0, n, body, 0)
    write((n - 1) * hb, hb).start()
    pltpu.make_async_copy(o_buf, o_hbm, w_sem.at[0]).wait()


@jax.jit
def pallas_standalone__mha_softmax__near_ridge_kernel(
    q: jax.Array,
    k: jax.Array,
    v: jax.Array,
):
    B, H, Sq, D = q.shape
    Sk, Dv = k.shape[2], v.shape[3]
    nh = B * H
    hb = _HEADS_PER_CHUNK if nh % _HEADS_PER_CHUNK == 0 else 1
    depth = _RING_DEPTH

    def kernel_function(*refs):
        _kernel(*refs, hb=hb, depth=depth, lead=_WRITE_LEAD)

    out = pl.pallas_call(
        kernel_function,
        in_specs=[pl.BlockSpec(memory_space=pl.ANY)] * 3,
        out_specs=pl.BlockSpec(memory_space=pl.ANY),
        out_shape=jax.ShapeDtypeStruct((nh, Sq, Dv), q.dtype),
        scratch_shapes=[
            pltpu.VMEM((depth, hb, Sq, D), q.dtype),
            pltpu.VMEM((depth, hb, Sk, D), k.dtype),
            pltpu.VMEM((depth, hb, Sk, Dv), v.dtype),
            pltpu.VMEM((nh, Sq, Dv), q.dtype),
            pltpu.SemaphoreType.DMA((3, depth)),
            pltpu.SemaphoreType.DMA((1,)),
        ],
        compiler_params=pltpu.CompilerParams(vmem_limit_bytes=64 * 1024 * 1024),
    )(q.reshape(nh, Sq, D), k.reshape(nh, Sk, D), v.reshape(nh, Sk, Dv))
    return out.reshape(B, H, Sq, Dv)
```

```python
import jax
import jax.numpy as jnp
import jax.experimental.pallas as pl
import jax.experimental.pallas.tpu as pltpu

_STREAMS = 4
_RING_DEPTH = 4
_PIECES = 4
_WRITE_LEAD = 2
_EARLY_HEADS = 8
_NT = (((1,), (1,)), ((), ()))


def _attention_head(q, k, v, scale):
    s = jax.lax.dot_general(q, k, _NT, preferred_element_type=jnp.float32)
    m = jnp.max(s, axis=-1, keepdims=True)
    p = jnp.exp((s - m) * scale)
    l = jnp.sum(p, axis=-1, keepdims=True)
    o = jnp.dot(p.astype(v.dtype), v, preferred_element_type=jnp.float32)
    return o * (1.0 / l)


def _kernel(q_hbm, k_hbm, v_hbm, o_hbm, in_buf, o_buf, r_sem, w_sem, *, pieces, lead, early):
    num_heads, seq, d = q_hbm.shape
    depth, _, streams = in_buf.shape[:3]
    n = num_heads // streams
    n_main = n - (depth - 1)
    rows = seq // pieces
    scale = d ** -0.5
    assert n_main > 0 and 0 < lead < depth
    assert early <= n - lead
    srcs = (q_hbm, k_hbm, v_hbm)

    read_order = [(j, s, p) for p in range(pieces) for j in range(3) for s in range(streams)]
    per_head = len(read_order) // streams

    def start_reads(step, slot, part):
        for t in range(part * per_head, (part + 1) * per_head):
            j, s, p = read_order[t]
            r = pl.ds(p * rows, rows)
            pltpu.make_async_copy(
                srcs[j].at[s * n + step, r], in_buf.at[slot, j, s, r], r_sem.at[slot]
            ).start(priority=t % 2)

    def wait_reads(slot):
        pltpu.make_async_copy(in_buf.at[slot], in_buf.at[slot], r_sem.at[slot]).wait()

    def start_writes(first, last):
        def one(c, carry):
            for p in range(pieces):
                r = pl.ds(p * rows, rows)
                for s in range(streams):
                    head = s * n + c
                    pltpu.make_async_copy(o_buf.at[head, r], o_hbm.at[head, r], w_sem.at[0]).start()
            return carry

        jax.lax.fori_loop(first, last, one, 0)

    def compute(step, slot, s):
        o = _attention_head(in_buf[slot, 0, s], in_buf[slot, 1, s], in_buf[slot, 2, s], scale)
        o_buf[s * n + step] = o.astype(o_buf.dtype)

    for i in range(depth - 1):
        for s in range(streams):
            start_reads(i, i, s)

    def main_step(i, carry):
        slot = jax.lax.rem(i, depth)
        nxt = i + depth - 1
        nxt_slot = jax.lax.rem(nxt, depth)
        wait_reads(slot)
        for s in range(streams):
            start_reads(nxt, nxt_slot, s)
            compute(i, slot, s)
        return carry

    def tail_step(i, carry):
        slot = jax.lax.rem(i, depth)
        wait_reads(slot)
        compute(i, slot, 0)

        @pl.when(i == n - lead)
        def _():
            start_writes(0, early)

        for s in range(1, streams):
            compute(i, slot, s)
        return carry

    jax.lax.fori_loop(0, n_main, main_step, 0)
    jax.lax.fori_loop(n_main, n, tail_step, 0)
    start_writes(early, n)
    pltpu.make_async_copy(o_buf, o_hbm, w_sem.at[0]).wait()


@jax.jit
def pallas_standalone__mha_softmax__near_ridge_kernel(
    q: jax.Array,
    k: jax.Array,
    v: jax.Array,
):
    B, H, S, D = q.shape
    assert k.shape == q.shape and v.shape == q.shape and k.dtype == q.dtype == v.dtype
    nh = B * H
    assert nh % _STREAMS == 0 and S % (16 * _PIECES) == 0

    def kernel_function(*refs):
        _kernel(*refs, pieces=_PIECES, lead=_WRITE_LEAD, early=_EARLY_HEADS)

    out = pl.pallas_call(
        kernel_function,
        in_specs=[pl.BlockSpec(memory_space=pl.ANY)] * 3,
        out_specs=pl.BlockSpec(memory_space=pl.ANY),
        out_shape=jax.ShapeDtypeStruct((nh, S, D), q.dtype),
        scratch_shapes=[
            pltpu.VMEM((_RING_DEPTH, 3, _STREAMS, S, D), q.dtype),
            pltpu.VMEM((nh, S, D), q.dtype),
            pltpu.SemaphoreType.DMA((_RING_DEPTH,)),
            pltpu.SemaphoreType.DMA((1,)),
        ],
        compiler_params=pltpu.CompilerParams(vmem_limit_bytes=64 * 1024 * 1024),
    )(q.reshape(nh, S, D), k.reshape(nh, S, D), v.reshape(nh, S, D))
    return out.reshape(B, H, S, D)
```
